```python
import jax
import jax.numpy as jnp

def _softmax(x, axis=-1):
    return jax.nn.softmax(x, axis=axis)
def _gelu(x):
    return jax.nn.gelu(x, approximate=True)
def _silu(x):
    return jax.nn.silu(x)
def _sigmoid(x):
    return jax.nn.sigmoid(x)
def _layernorm(x, axis=-1, eps=1e-5):
    m = jnp.mean(x, axis=axis, keepdims=True)
    v = jnp.var(x, axis=axis, keepdims=True)
    return (x - m) / jnp.sqrt(v + eps)
def _scatter_add(tgt, idx, src, axis=0):
    return tgt.at[idx].add(src)
def _segment_sum(src, seg, n):
    return jax.ops.segment_sum(src, seg, n)
class _Rng:
    def __init__(self, key):
        self._k = key
    def _next(self):
        self._k, sub = jax.random.split(self._k)
        return sub
    def normal(self, shape):
        return jax.random.normal(self._next(), shape, dtype=jnp.bfloat16)
    def randint(self, lo, hi, shape):
        return jax.random.randint(self._next(), shape, lo, hi, dtype=jnp.int32)
    def uniform(self, shape, lo=0.0, hi=1.0):
        return jax.random.uniform(self._next(), shape, jnp.bfloat16, lo, hi)
    def permutation(self, n):
        return jax.random.permutation(self._next(), n)


kernel_name = 'standalone__cross_network_dcn_v2__recsys'

def setup_inputs():
    _rng = _Rng(jax.random.key(int.from_bytes(__import__("os").urandom(4), "little")))
    _w = (lambda a: (lambda t: t.astype(jnp.bfloat16) if jnp.issubdtype(t.dtype, jnp.floating) else t)(jnp.asarray(a)))
    B, F, D, L = 16384, 100, 16, 3
    Din = min(F * D, 512)
    R = max(Din // 4, 2)
    sc = Din ** -0.5
    return {
        "x0": _w((lambda *s: _rng.normal(s) * 0.05)(B, Din)),
        "U":  _w((lambda *s: _rng.normal(s) * 0.05)(L, Din, R) * sc),
        "V":  _w((lambda *s: _rng.normal(s) * 0.05)(L, R, Din) * sc),
        "bs": _w((lambda *s: _rng.normal(s) * 0.05)(L, Din)),
    }

def reference(x0, U, V, bs):
    x = x0
    for l in range(U.shape[0]):
        h = jnp.einsum('rd,bd->br', V[l], x)
        h = jnp.einsum('dr,br->bd', U[l], h)
        x = x0 * (h + bs[l]) + x
    return x
```

```python
import functools

import jax
import jax.numpy as jnp
import jax.experimental.pallas as pl
import jax.experimental.pallas.tpu as pltpu

_NT = (((1,), (1,)), ((), ()))


def _cross_kernel(x0_ref, u_ref, v_ref, b_ref, o_ref, *, n_layers, chunk):
    bm = x0_ref.shape[0]
    for c in range(bm // chunk):
        rows = pl.ds(c * chunk, chunk)
        x0b = x0_ref[rows, :]
        x0 = x0b.astype(jnp.float32)
        x = x0
        xb = x0b
        for l in range(n_layers):
            h = jax.lax.dot_general(xb, v_ref[l], _NT,
                                    preferred_element_type=jnp.float32)
            g = jax.lax.dot_general(h.astype(jnp.bfloat16), u_ref[l], _NT,
                                    preferred_element_type=jnp.float32)
            x = x0 * (g + b_ref[pl.ds(l, 1), :].astype(jnp.float32)) + x
            xb = x.astype(jnp.bfloat16)
        o_ref[rows, :] = xb


@jax.jit
def pallas_standalone__cross_network_dcn_v2__recsys_kernel(
    x0: jax.Array,
    U: jax.Array,
    V: jax.Array,
    bs: jax.Array,
):
    B, D = x0.shape
    L, _, R = U.shape
    bm = 1024
    chunk = 512
    return pl.pallas_call(
        functools.partial(_cross_kernel, n_layers=L, chunk=chunk),
        grid=(B // bm,),
        in_specs=[
            pl.BlockSpec((bm, D), lambda i: (i, 0)),
            pl.BlockSpec((L, D, R), lambda i: (0, 0, 0)),
            pl.BlockSpec((L, R, D), lambda i: (0, 0, 0)),
            pl.BlockSpec((L, D), lambda i: (0, 0)),
        ],
        out_specs=pl.BlockSpec((bm, D), lambda i: (i, 0)),
        out_shape=jax.ShapeDtypeStruct((B, D), x0.dtype),
        compiler_params=pltpu.CompilerParams(
            dimension_semantics=("arbitrary",),
            vmem_limit_bytes=64 * 1024 * 1024,
        ),
    )(x0, U, V, bs)
```

```python
import functools

import jax
import jax.numpy as jnp
import jax.experimental.pallas as pl
import jax.experimental.pallas.tpu as pltpu

_NT = (((1,), (1,)), ((), ()))

_HEAD = ((256,), (512, 256), (512,) * 4 + (256,))
_BODY = (512,) * 8 + (256,)
_OUT_AFTER = (4, 6, 7, 8)


def _cross_kernel(x_hbm, u_hbm, v_hbm, b_hbm, o_hbm,
                  x_vmem, o_vmem, u_vmem, v_vmem, b_vmem, in_sems, out_sems,
                  *, n_layers, head, n_body, body, out_after):
    head_rows = sum(sum(blk) for blk in head)
    body_rows = sum(body)

    def rows(start, size):
        if not isinstance(start, int):
            start = pl.multiple_of(start, 128)
        return pl.ds(start, size)

    def in_copy(k, start, size):
        r = rows(start, size)
        return pltpu.make_async_copy(x_hbm.at[r], x_vmem.at[r], in_sems.at[k])

    def out_copy(k, start, size):
        r = rows(start, size)
        return pltpu.make_async_copy(o_vmem.at[r], o_hbm.at[r], out_sems.at[k])

    def cross(start, size):
        r = rows(start, size)
        x = x_vmem[r, :]
        for l in range(n_layers):
            h = jax.lax.dot_general(x, v_vmem[l], _NT,
                                    preferred_element_type=jnp.float32)
            g = jax.lax.dot_general(h.astype(x.dtype), u_vmem[l], _NT,
                                    preferred_element_type=jnp.float32)
            bias = b_vmem[pl.ds(l, 1), :].astype(jnp.float32)
            x0 = x_vmem[r, :].astype(jnp.float32)
            x = (x0 * (g + bias) + x.astype(jnp.float32)).astype(x.dtype)
        o_vmem[r, :] = x

    n_blocks = len(head) + n_body
    weights = [
        pltpu.make_async_copy(src, dst, in_sems.at[n_blocks + i])
        for i, (src, dst) in enumerate(
            ((b_hbm, b_vmem), (v_hbm, v_vmem), (u_hbm, u_vmem)))
    ]
    head_start = [0]
    for blk in head:
        head_start.append(head_start[-1] + sum(blk))
    offs = [0]
    for size in body:
        offs.append(offs[-1] + size)
    groups = list(zip((0,) + tuple(j + 1 for j in out_after[:-1]), out_after))

    for w in weights:
        w.start()
    for k, blk in enumerate(head):
        in_copy(k, head_start[k], sum(blk)).start()
    for i in range(n_body):
        in_copy(len(head) + i, head_rows + i * body_rows, body_rows).start()
    for w in weights:
        w.wait()

    for k, blk in enumerate(head):
        in_copy(k, head_start[k], sum(blk)).wait()
        start = head_start[k]
        for size in blk:
            cross(start, size)
            start += size
    head_out = out_copy(n_body * len(groups), 0, head_rows)
    head_out.start()

    def group_copy(i, g):
        first, last = groups[g]
        return out_copy(i * len(groups) + g,
                        head_rows + i * body_rows + offs[first],
                        offs[last + 1] - offs[first])

    def body_step(i, carry):
        base = head_rows + i * body_rows
        in_copy(len(head) + i, base, body_rows).wait()
        for j, size in enumerate(body):
            cross(base + offs[j], size)
            if j in out_after:
                group_copy(i, out_after.index(j)).start()
        return carry

    jax.lax.fori_loop(0, n_body, body_step, 0)

    head_out.wait()
    for i in range(n_body):
        for g in range(len(groups)):
            group_copy(i, g).wait()


@jax.jit
def pallas_standalone__cross_network_dcn_v2__recsys_kernel(
    x0: jax.Array,
    U: jax.Array,
    V: jax.Array,
    bs: jax.Array,
):
    B, D = x0.shape
    L = U.shape[0]
    head_rows = sum(sum(blk) for blk in _HEAD)
    n_body, rem = divmod(B - head_rows, sum(_BODY))
    assert n_body >= 1 and rem == 0, "row schedule does not cover the batch"
    return pl.pallas_call(
        functools.partial(_cross_kernel, n_layers=L, head=_HEAD, n_body=n_body,
                          body=_BODY, out_after=_OUT_AFTER),
        in_specs=[pl.BlockSpec(memory_space=pl.ANY)] * 4,
        out_specs=pl.BlockSpec(memory_space=pl.ANY),
        out_shape=jax.ShapeDtypeStruct((B, D), x0.dtype),
        scratch_shapes=[
            pltpu.VMEM((B, D), x0.dtype),
            pltpu.VMEM((B, D), x0.dtype),
            pltpu.VMEM(U.shape, U.dtype),
            pltpu.VMEM(V.shape, V.dtype),
            pltpu.VMEM(bs.shape, bs.dtype),
            pltpu.SemaphoreType.DMA((len(_HEAD) + n_body + 3,)),
            pltpu.SemaphoreType.DMA((n_body * len(_OUT_AFTER) + 1,)),
        ],
        compiler_params=pltpu.CompilerParams(
            vmem_limit_bytes=100 * 1024 * 1024),
    )(x0, U, V, bs)
```

```python
import functools

import jax
import jax.numpy as jnp
import jax.experimental.pallas as pl
import jax.experimental.pallas.tpu as pltpu

_NT = (((1,), (1,)), ((), ()))

_CHUNKS = (288, 256, 256) + (512,) * 13 + (256, 256, 224)
_IN_STARTS = (0, 1, 2, 3, 5, 9)
_OUT_ENDS = (9, 13, 15, 16, 17)
_LAST_CUTS = (112, 176)
_PIN_ROW = 48
_SPARE = 16


def _cross_kernel(x_hbm, u_hbm, v_hbm, b_hbm, o_hbm,
                  x_vmem, o_vmem, u_vmem, v_vmem, b_vmem, sems, *, n_steps):
    batch, dim = x_hbm.shape
    n_layers, rank, _ = v_hbm.shape
    offs = [sum(_CHUNKS[:j]) for j in range(len(_CHUNKS) + 1)]
    step_rows = offs[-1]
    in_offs = [offs[j] for j in _IN_STARTS] + [step_rows]
    n_in = len(_IN_STARTS)

    x_sems = (0, 2 * n_layers, 2)
    out_sem = 1

    def v_copy(l):
        return pltpu.make_async_copy(
            v_hbm.at[l], v_vmem.at[l, pl.ds(0, rank)], sems.at[2 * l])

    def u_copy(l):
        return pltpu.make_async_copy(
            u_hbm.at[l], u_vmem.at[l, pl.ds(0, dim)], sems.at[2 * l + 1])

    def x_copy(p):
        step, k = divmod(p, n_in)
        r = pl.ds(step * step_rows + in_offs[k], in_offs[k + 1] - in_offs[k])
        return pltpu.make_async_copy(
            x_hbm.at[r], x_vmem.at[r], sems.at[x_sems[p % len(x_sems)]])

    def out_copy(start, size):
        r = pl.ds(start, size)
        return pltpu.make_async_copy(o_vmem.at[r], o_hbm.at[r], sems.at[out_sem])

    def pin(spare_ref, value):
        spare_ref[...] = value

    b_copy = pltpu.make_async_copy(b_hbm, b_vmem, sems.at[0])
    b_copy.start()
    v_copy(0).start()
    x_copy(0).start()
    u_copy(0).start()
    for l in range(1, n_layers):
        v_copy(l).start()
        u_copy(l).start()
    x_copy(1).start()
    b_copy.wait()
    v_copy(0).wait()
    x_copy(0).wait()

    def step_body(i, carry):
        def on_step(step, fn):
            pl.when(i == step)(fn)

        out_lo = 0
        for j, size in enumerate(_CHUNKS):
            last = j == len(_CHUNKS) - 1

            def rows(lo, hi, j=j):
                start = pl.multiple_of(i * step_rows + offs[j] + lo, 16)
                return pl.ds(start, hi - lo)

            x = x_vmem[rows(0, size), :]
            for l in range(n_layers):
                h = jax.lax.dot_general(
                    x, v_vmem[l, pl.ds(0, rank)], _NT,
                    preferred_element_type=jnp.float32).astype(x.dtype)
                if j == 0:
                    pin(u_vmem.at[l, pl.ds(dim, _SPARE)],
                        h[_PIN_ROW:_PIN_ROW + _SPARE])
                    on_step(0, u_copy(l).wait)
                u = u_vmem[l, pl.ds(0, dim)]
                if l == n_layers - 1 and (last or j + 1 in _IN_STARTS):
                    k = n_in if last else _IN_STARTS.index(j + 1)
                    pin(x_vmem.at[pl.ds(batch, _SPARE), pl.ds(0, rank)],
                        h[size - _SPARE:])
                    for step in range(n_steps):
                        p = step * n_in + k
                        if p < n_steps * n_in:
                            on_step(step, x_copy(p).wait)
                        if p + 2 < n_steps * n_in:
                            on_step(step, x_copy(p + 2).start)
                g = jax.lax.dot_general(
                    h, u, _NT, preferred_element_type=jnp.float32)

                cuts = _LAST_CUTS if last and l == n_layers - 1 else ()
                for lo, hi in zip((0,) + cuts, cuts + (size,)):
                    x0 = x_vmem[rows(lo, hi), :].astype(jnp.float32)
                    bias = b_vmem[pl.ds(l, 1), :].astype(jnp.float32)
                    y = x0 * (g[lo:hi] + bias) + x[lo:hi].astype(jnp.float32)
                    y = y.astype(x.dtype)
                    if l == n_layers - 1:
                        o_vmem[rows(lo, hi), :] = y
                        if last or j in _OUT_ENDS:
                            out_hi = offs[j] + hi
                            for step in range(n_steps):
                                on_step(step, out_copy(
                                    step * step_rows + out_lo,
                                    out_hi - out_lo).start)
                            out_lo = out_hi
                x = y
                if j == 0 and l + 1 < n_layers:
                    pin(v_vmem.at[l + 1, pl.ds(rank, _SPARE)],
                        x[_PIN_ROW:_PIN_ROW + _SPARE])
                    on_step(0, v_copy(l + 1).wait)
                    if l == 0:
                        on_step(0, x_copy(2).start)
        return carry

    jax.lax.fori_loop(0, n_steps, step_body, 0)
    pltpu.make_async_copy(o_vmem, o_hbm, sems.at[out_sem]).wait()


@jax.jit
def pallas_standalone__cross_network_dcn_v2__recsys_kernel(
    x0: jax.Array,
    U: jax.Array,
    V: jax.Array,
    bs: jax.Array,
):
    B, D = x0.shape
    L, _, R = U.shape
    n_steps, rem = divmod(B, sum(_CHUNKS))
    assert rem == 0 and L >= 2, "row schedule does not fit these shapes"
    return pl.pallas_call(
        functools.partial(_cross_kernel, n_steps=n_steps),
        in_specs=[pl.BlockSpec(memory_space=pl.ANY)] * 4,
        out_specs=pl.BlockSpec(memory_space=pl.ANY),
        out_shape=jax.ShapeDtypeStruct((B, D), x0.dtype),
        scratch_shapes=[
            pltpu.VMEM((B + _SPARE, D), x0.dtype),
            pltpu.VMEM((B, D), x0.dtype),
            pltpu.VMEM((L, D + _SPARE, R), U.dtype),
            pltpu.VMEM((L, R + _SPARE, D), V.dtype),
            pltpu.VMEM(bs.shape, bs.dtype),
            pltpu.SemaphoreType.DMA((2 * L + 1,)),
        ],
        compiler_params=pltpu.CompilerParams(
            vmem_limit_bytes=64 * 1024 * 1024,
            flags={"XLA_TPU_RESCHEDULE_DMA_DONES": True},
        ),
    )(x0, U, V, bs)
```

```python
import functools

import jax
import jax.numpy as jnp
import jax.experimental.pallas as pl
import jax.experimental.pallas.tpu as pltpu

_NT = (((1,), (1,)), ((), ()))

_CHUNKS = (272, 192, 304) + (512,) * 13 + (256, 352, 160)
_IN_STARTS = (0, 1, 2, 3, 5, 9)
_OUT_ENDS = (9, 13, 15, 16, 17)
_LAST_CUTS = (48, 96, 128)
_WEIGHT_PIN_ROW = 48
_ROWS_PIN_LEAD = 192
_SPARE = 16


def _cross_kernel(x_hbm, u_hbm, v_hbm, b_hbm, o_hbm,
                  x_vmem, o_vmem, u_vmem, v_vmem, b_vmem, sems, *, n_steps):
    batch, dim = x_hbm.shape
    n_layers, rank, _ = v_hbm.shape
    offs = [sum(_CHUNKS[:j]) for j in range(len(_CHUNKS) + 1)]
    step_rows = offs[-1]
    in_offs = [offs[j] for j in _IN_STARTS] + [step_rows]
    n_in = len(_IN_STARTS)

    out_sem = 1

    def v_copy(l):
        return pltpu.make_async_copy(
            v_hbm.at[l], v_vmem.at[l, pl.ds(0, rank)], sems.at[2 * l])

    def u_copy(l):
        return pltpu.make_async_copy(
            u_hbm.at[l], u_vmem.at[l, pl.ds(0, dim)], sems.at[2 * l + 1])

    def x_copy(p):
        step, k = divmod(p, n_in)
        r = pl.ds(step * step_rows + in_offs[k], in_offs[k + 1] - in_offs[k])
        sem = 2 * ((p - 1) % n_layers) if p else 0
        return pltpu.make_async_copy(x_hbm.at[r], x_vmem.at[r], sems.at[sem])

    def out_copy(start, size):
        r = pl.ds(start, size)
        return pltpu.make_async_copy(o_vmem.at[r], o_hbm.at[r], sems.at[out_sem])

    def pin(spare_ref, value):
        spare_ref[...] = value

    b_copy = pltpu.make_async_copy(b_hbm, b_vmem, sems.at[1])
    v_copy(0).start()
    x_copy(0).start()
    u_copy(0).start()
    b_copy.start()
    for l in range(1, n_layers):
        v_copy(l).start()
        u_copy(l).start()
    v_copy(0).wait()
    x_copy(0).wait()
    x_copy(1).start()

    def step_body(i, carry):
        def on_step(step, fn):
            pl.when(i == step)(fn)

        out_lo = 0
        v_next = None
        for j, size in enumerate(_CHUNKS):
            last = j == len(_CHUNKS) - 1

            def rows(lo, hi, j=j):
                start = pl.multiple_of(i * step_rows + offs[j] + lo, 16)
                return pl.ds(start, hi - lo)

            x = x_vmem[rows(0, size), :]
            for l in range(n_layers):
                v = v_vmem[l, pl.ds(0, rank)] if v_next is None else v_next
                v_next = None
                h = jax.lax.dot_general(
                    x, v, _NT, preferred_element_type=jnp.float32)
                h = h.astype(x.dtype)
                if j == 0:
                    pin(u_vmem.at[l, pl.ds(dim, _SPARE)],
                        h[_WEIGHT_PIN_ROW:_WEIGHT_PIN_ROW + _SPARE])
                    on_step(0, u_copy(l).wait)
                    if l == 0:
                        on_step(0, b_copy.wait)
                g = jax.lax.dot_general(
                    h, u_vmem[l, pl.ds(0, dim)], _NT,
                    preferred_element_type=jnp.float32)

                final = l == n_layers - 1
                out_cuts, in_cut = (), None
                if final and last:
                    out_cuts, in_cut = _LAST_CUTS + (size,), _SPARE
                elif final:
                    out_cuts = (size,) if j in _OUT_ENDS else ()
                    if j + 1 in _IN_STARTS:
                        in_cut = max(_SPARE, size - _ROWS_PIN_LEAD)
                        v_next = v_vmem[0, pl.ds(0, rank)]
                cuts = sorted({size, *out_cuts, in_cut or size})
                for lo, hi in zip([0] + cuts, cuts):
                    x0 = x_vmem[rows(lo, hi), :].astype(jnp.float32)
                    bias = b_vmem[pl.ds(l, 1), :].astype(jnp.float32)
                    y = x0 * (g[lo:hi] + bias) + x[lo:hi].astype(jnp.float32)
                    y = y.astype(x.dtype)
                    if final:
                        o_vmem[rows(lo, hi), :] = y
                    if hi in out_cuts:
                        out_hi = offs[j] + hi
                        for step in range(n_steps):
                            on_step(step, out_copy(step * step_rows + out_lo,
                                                   out_hi - out_lo).start)
                        out_lo = out_hi
                    if hi == in_cut:
                        k = n_in if last else _IN_STARTS.index(j + 1)
                        pin(x_vmem.at[pl.ds(batch, _SPARE), pl.ds(0, rank)],
                            y[hi - lo - _SPARE:, :rank])
                        for step in range(n_steps):
                            p = step * n_in + k
                            if p < n_steps * n_in:
                                on_step(step, x_copy(p).wait)
                            if p + n_layers < n_steps * n_in:
                                on_step(step, x_copy(p + n_layers).start)
                x = y
                if j == 0 and not final:
                    pin(v_vmem.at[l + 1, pl.ds(rank, _SPARE)],
                        x[_WEIGHT_PIN_ROW:_WEIGHT_PIN_ROW + _SPARE])
                    on_step(0, v_copy(l + 1).wait)
                    on_step(0, x_copy(l + 2).start)
        return carry

    jax.lax.fori_loop(0, n_steps, step_body, 0)
    pltpu.make_async_copy(o_vmem, o_hbm, sems.at[out_sem]).wait()


@jax.jit
def pallas_standalone__cross_network_dcn_v2__recsys_kernel(
    x0: jax.Array,
    U: jax.Array,
    V: jax.Array,
    bs: jax.Array,
):
    B, D = x0.shape
    L, _, R = U.shape
    n_steps, rem = divmod(B, sum(_CHUNKS))
    assert rem == 0 and L < n_steps * len(_IN_STARTS), "schedule does not fit"
    return pl.pallas_call(
        functools.partial(_cross_kernel, n_steps=n_steps),
        in_specs=[pl.BlockSpec(memory_space=pl.ANY)] * 4,
        out_specs=pl.BlockSpec(memory_space=pl.ANY),
        out_shape=jax.ShapeDtypeStruct((B, D), x0.dtype),
        scratch_shapes=[
            pltpu.VMEM((B + _SPARE, D), x0.dtype),
            pltpu.VMEM((B, D), x0.dtype),
            pltpu.VMEM((L, D + _SPARE, R), U.dtype),
            pltpu.VMEM((L, R + _SPARE, D), V.dtype),
            pltpu.VMEM(bs.shape, bs.dtype),
            pltpu.SemaphoreType.DMA((2 * L,)),
        ],
        compiler_params=pltpu.CompilerParams(
            vmem_limit_bytes=64 * 1024 * 1024,
            flags={"XLA_TPU_RESCHEDULE_DMA_DONES": True},
        ),
    )(x0, U, V, bs)
```
